```python
import os as _os
_os.environ.setdefault("JAX_PLATFORMS", "cpu")
import jax
import jax.numpy as jnp

def _softmax(x, axis=-1):
    return jax.nn.softmax(x, axis=axis)
def _gelu(x):
    return jax.nn.gelu(x, approximate=True)
def _silu(x):
    return jax.nn.silu(x)
def _sigmoid(x):
    return jax.nn.sigmoid(x)
def _layernorm(x, axis=-1, eps=1e-5):
    m = jnp.mean(x, axis=axis, keepdims=True)
    v = jnp.var(x, axis=axis, keepdims=True)
    return (x - m) / jnp.sqrt(v + eps)
def _scatter_add(tgt, idx, src, axis=0):
    return tgt.at[idx].add(src)
def _segment_sum(src, seg, n):
    return jax.ops.segment_sum(src, seg, n)
class _Rng:
    def __init__(self, key):
        self._k = key
    def _next(self):
        self._k, sub = jax.random.split(self._k)
        return sub
    def normal(self, shape):
        return jax.random.normal(self._next(), shape, dtype=jnp.bfloat16)
    def randint(self, lo, hi, shape):
        return jax.random.randint(self._next(), shape, lo, hi, dtype=jnp.int32)
    def uniform(self, shape, lo=0.0, hi=1.0):
        return jax.random.uniform(self._next(), shape, jnp.bfloat16, lo, hi)
    def permutation(self, n):
        return jax.random.permutation(self._next(), n)


kernel_name = 'parallel_sum__softmax_full_mha__swiglu_ffn__prompt'

def setup_inputs():
    _rng = _Rng(jax.random.key(int.from_bytes(__import__("os").urandom(4), "little")))
    _w = (lambda a: (lambda t: t.astype(jnp.bfloat16) if jnp.issubdtype(t.dtype, jnp.floating) else t)(jnp.asarray(a)))
    def _A_setup():
        B, S, D = 1, 2048, 640
        return {
            "x": _w((lambda *s: _rng.normal(s) * 0.05)(B, S, D)),
            "wqkv": _w((lambda *s: _rng.normal(s) * 0.1)(D, 3 * D)),
            "wo": _w((lambda *s: _rng.normal(s) * 0.05)(D, D)),
        }
    _A_in = _A_setup()

    def _B_setup():
        B, S, D, F = 1, 2048, 640, 1536
        return {
            "x": _w((lambda *s: _rng.normal(s) * 0.05)(B, S, D)),
            "w_gate": _w((lambda *s: _rng.normal(s) * 0.05)(D, F)),
            "w_up": _w((lambda *s: _rng.normal(s) * 0.05)(D, F)),
            "w_down": _w((lambda *s: _rng.normal(s) * 0.05)(F, D)),
        }
    _B_in = _B_setup()

    return {
        "A_x": _A_in["x"],
        "A_wqkv": _A_in["wqkv"],
        "A_wo": _A_in["wo"],
        "B_x": _B_in["x"],
        "B_w_gate": _B_in["w_gate"],
        "B_w_up": _B_in["w_up"],
        "B_w_down": _B_in["w_down"],
    }

def reference(A_x, A_wqkv, A_wo, B_x, B_w_gate, B_w_up, B_w_down):
    def _A_ref(x, wqkv, wo):
        B, S, D = x.shape
        H = 32; Dh = D // H
        qkv = (lambda x, *d: x.transpose(*d))((x @ wqkv).reshape(B, S, 3, H, Dh), 2, 0, 3, 1, 4)
        q, k, v = qkv[0], qkv[1], qkv[2]
        scale = Dh ** -0.5
        scores = jnp.einsum("bhqd,bhkd->bhqk", q, k) * scale
        p = _softmax(scores, axis=-1)
        o = jnp.einsum("bhqk,bhkd->bhqd", p, v)
        return (lambda x, *d: x.transpose(*d))(o, 0, 2, 1, 3).reshape(B, S, D) @ wo

    def _B_ref(x, w_gate, w_up, w_down):
        g = _silu(x @ w_gate)
        u = x @ w_up
        return (g * u) @ w_down

    x = A_x
    xn = _layernorm(x, axis=-1)
    return x + _A_ref(xn, A_wqkv, A_wo) + _B_ref(xn, B_w_gate, B_w_up, B_w_down)
```

```python
import math

import jax
import jax.numpy as jnp
import jax.experimental.pallas as pl
import jax.experimental.pallas.tpu as pltpu

S, D, F, H = 2048, 640, 1536, 32
DH = D // H
LANES = 128
BQ = 512
BK = 128
NQ = S // BQ
NG = D // LANES
NGS = 2 * NG - 1
MV = 24
BF = 512
EPS = 1e-5
Q_SCALE = DH ** -0.5 * math.log2(math.e)

F32 = jnp.float32
BF16 = jnp.bfloat16
NT = (((1,), (1,)), ((), ()))


def _dot(a, b):
    return jax.lax.dot_general(a, b, (((1,), (0,)), ((), ())), preferred_element_type=F32)


def _kernel(x_hbm, wqkv_hbm, wo_hbm, wg_hbm, wu_hbm, wd_hbm, out_hbm,
            x_v, wqkv_v, wo_v, wg_v, wu_v, wd_v, xn_v, wt_v, kg_v, qt_v, vt_v,
            s_v, m_v, ot_v, out_v, x_sem, w_sem, o_sem):

    def x_copy(r):
        rows = pl.ds(r * BQ, BQ)
        return pltpu.make_async_copy(x_hbm.at[rows], x_v.at[rows], x_sem.at[r])

    def qkv_copy(i):
        cols = pl.ds(i * D, D)
        return pltpu.make_async_copy(wqkv_hbm.at[:, cols], wqkv_v.at[:, cols], w_sem.at[i])

    late_copies = [
        pltpu.make_async_copy(src, dst, w_sem.at[3 + i])
        for i, (src, dst) in enumerate(
            [(wg_hbm, wg_v), (wu_hbm, wu_v), (wd_hbm, wd_v), (wo_hbm, wo_v)])
    ]

    def out_copy(r):
        rows = pl.ds(pl.multiple_of(r * BF, BF), BF)
        return pltpu.make_async_copy(out_v.at[rows], out_hbm.at[rows], o_sem.at[r])

    x_copy(0).start()
    qkv_copy(1).start()
    for r in range(1, NQ):
        x_copy(r).start()
    qkv_copy(0).start()
    qkv_copy(2).start()
    for c in late_copies:
        c.start()

    qkv_copy(1).wait()

    def ln_k(r, carry):
        x_copy(r).wait()
        rows = pl.ds(pl.multiple_of(r * BQ, BQ), BQ)
        x = x_v[rows, :].astype(F32)
        mean = jnp.sum(x, axis=1, keepdims=True) * (1.0 / D)
        xc = x - mean
        var = jnp.sum(xc * xc, axis=1, keepdims=True) * (1.0 / D)
        xn = (xc * jax.lax.rsqrt(var + EPS)).astype(BF16)
        xn_v[rows, :] = xn
        k = _dot(xn, wqkv_v[:, D:2 * D])
        upper = jax.lax.broadcasted_iota(jnp.int32, (BQ, LANES), 1) >= LANES // 2
        for g in range(NG):
            kg = k[:, g * LANES:(g + 1) * LANES]
            kg_v[2 * g, rows, :] = kg.astype(BF16)
            if g + 1 < NG:
                nxt = k[:, (g + 1) * LANES:(g + 2) * LANES]
                kg_v[2 * g + 1, rows, :] = jnp.where(upper, kg, nxt).astype(BF16)
        return carry

    jax.lax.fori_loop(0, NQ, ln_k, 0)

    qkv_copy(0).wait()
    qkv_copy(2).wait()
    for i in range(NG):
        wt_v[i * LANES:(i + 1) * LANES, :] = wqkv_v[:, i * LANES:(i + 1) * LANES].T
        wt_v[D + i * LANES:D + (i + 1) * LANES, :] = (
            wqkv_v[:, 2 * D + i * LANES:2 * D + (i + 1) * LANES].T)

    def q_v(r, carry):
        rows = pl.ds(pl.multiple_of(r * BQ, BQ), BQ)
        xn = xn_v[rows, :]
        qt = jax.lax.dot_general(wt_v[0:D, :], xn, NT, preferred_element_type=F32) * Q_SCALE
        upper = jax.lax.broadcasted_iota(jnp.int32, (LANES, BQ), 0) >= LANES // 2
        for g in range(NG):
            qg = qt[g * LANES:(g + 1) * LANES, :]
            qt_v[r, 2 * g] = qg.astype(BF16)
            if g + 1 < NG:
                nxt = qt[(g + 1) * LANES:(g + 2) * LANES, :]
                qt_v[r, 2 * g + 1] = jnp.where(upper, qg, nxt).astype(BF16)
        vt = jax.lax.dot_general(wt_v[D:2 * D, :], xn, NT, preferred_element_type=F32)
        vt = vt.astype(BF16).astype(F32)
        low = jax.lax.broadcasted_iota(jnp.int32, (8, BQ), 0) < 4
        for p in range(H // 2):
            b = 2 * DH * p
            mid = vt[b + 16:b + 24, :]
            vt_v[r, 2 * p, 0:16, :] = vt[b:b + 16, :]
            vt_v[r, 2 * p, 16:24, :] = jnp.where(low, mid, 1.0)
            vt_v[r, 2 * p + 1, 0:8, :] = jnp.where(low, 1.0, mid)
            vt_v[r, 2 * p + 1, 8:24, :] = vt[b + 24:b + 40, :]
        return carry

    jax.lax.fori_loop(0, NQ, q_v, 0)

    def head_operands(qb, h):
        lo = h * DH
        start = lo & (LANES - 1)
        gid = 2 * (lo >> 7) + (start > LANES - DH).astype(jnp.int32)
        row = jax.lax.broadcasted_iota(jnp.int32, (LANES, BQ), 0)
        mine = ((row - start) & (LANES - 1)) < DH
        qm = jnp.where(mine, qt_v[qb, gid].astype(F32), 0.0).astype(BF16)
        return gid, qm

    def scores_chunk(c, gid, qm):
        keys = pl.ds(c * BK, BK)
        st = _dot(kg_v[gid, keys, :], qm)
        s_v[keys, :] = st
        return jnp.max(st.reshape(BK // 8, 8, BQ), axis=0)

    def stage(h, nxt):
        m = jnp.max(m_v[...], axis=0, keepdims=True)
        if nxt is not None:
            gid, qm = head_operands(*nxt)
        mx = acc = None
        for c in range(S // BK):
            s = s_v[pl.ds(c * BK, BK), :]
            if nxt is not None:
                t = scores_chunk(c, gid, qm)
                mx = t if mx is None else jnp.maximum(mx, t)
            p = jnp.exp2(s - m).astype(BF16)
            r, off = divmod(c * BK, BQ)
            d = _dot(vt_v[r, h, :, off:off + BK], p)
            acc = d if acc is None else acc + d
        if nxt is not None:
            m_v[...] = mx
        return acc

    gid0, qm0 = head_operands(0, jnp.int32(0))
    mx0 = None
    for c in range(S // BK):
        t0 = scores_chunk(c, gid0, qm0)
        mx0 = t0 if mx0 is None else jnp.maximum(mx0, t0)
    m_v[...] = mx0

    n_pairs = NQ * H // 2

    def pair(t, carry):
        qb, p = t >> 4, t & (H // 2 - 1)
        t1 = jnp.minimum(t + 1, n_pairs - 1)
        oa = stage(2 * p, (qb, 2 * p + 1))
        ob = stage(2 * p + 1, (t1 >> 4, 2 * (t1 & (H // 2 - 1))))
        oa = oa * (1.0 / oa[20:21, :])
        ob = ob * (1.0 / ob[0:1, :])
        low = jax.lax.broadcasted_iota(jnp.int32, (8, BQ), 0) < 4
        base = pl.multiple_of(p * 2 * DH, 8)
        ot_v[qb, pl.ds(base, 16), :] = oa[0:16]
        ot_v[qb, pl.ds(base + 16, 8), :] = jnp.where(low, oa[16:24], ob[0:8])
        ot_v[qb, pl.ds(base + 24, 16), :] = ob[8:24]
        return carry

    jax.lax.fori_loop(0, n_pairs, pair, 0)

    for c in late_copies:
        c.wait()

    def finish(r, carry):
        rows = pl.ds(pl.multiple_of(r * BF, BF), BF)
        xn = xn_v[rows, :]
        g = _dot(xn, wg_v[...])
        u = _dot(xn, wu_v[...])
        hid = (g * jax.nn.sigmoid(g) * u).astype(BF16)
        o = ot_v[r].T.astype(BF16)
        y = x_v[rows, :].astype(F32) + _dot(o, wo_v[...]) + _dot(hid, wd_v[...])
        out_v[rows, :] = y.astype(BF16)
        out_copy(r).start()
        return carry

    jax.lax.fori_loop(0, S // BF, finish, 0)
    for r in range(S // BF):
        out_copy(r).wait()


@jax.jit
def pallas_parallel_sum__softmax_full_mha__swiglu_ffn__prompt_kernel(
    A_x: jax.Array,
    A_wqkv: jax.Array,
    A_wo: jax.Array,
    B_x: jax.Array,
    B_w_gate: jax.Array,
    B_w_up: jax.Array,
    B_w_down: jax.Array,
):
    del B_x
    hbm = pl.BlockSpec(memory_space=pl.ANY)
    out = pl.pallas_call(
        _kernel,
        out_shape=jax.ShapeDtypeStruct((S, D), BF16),
        in_specs=[hbm] * 6,
        out_specs=hbm,
        scratch_shapes=[
            pltpu.VMEM((S, D), BF16),
            pltpu.VMEM((D, 3 * D), BF16),
            pltpu.VMEM((D, D), BF16),
            pltpu.VMEM((D, F), BF16),
            pltpu.VMEM((D, F), BF16),
            pltpu.VMEM((F, D), BF16),
            pltpu.VMEM((S, D), BF16),
            pltpu.VMEM((2 * D, D), BF16),
            pltpu.VMEM((NGS, S, LANES), BF16),
            pltpu.VMEM((NQ, NGS, LANES, BQ), BF16),
            pltpu.VMEM((NQ, H, MV, BQ), F32),
            pltpu.VMEM((S, BQ), F32),
            pltpu.VMEM((8, BQ), F32),
            pltpu.VMEM((NQ, D, BQ), F32),
            pltpu.VMEM((S, D), BF16),
            pltpu.SemaphoreType.DMA((NQ,)),
            pltpu.SemaphoreType.DMA((7,)),
            pltpu.SemaphoreType.DMA((S // BF,)),
        ],
        compiler_params=pltpu.CompilerParams(vmem_limit_bytes=100 * 2**20),
    )(A_x.reshape(S, D), A_wqkv, A_wo, B_w_gate, B_w_up, B_w_down)
    return out.reshape(1, S, D)
```

```python
import math

import jax
import jax.numpy as jnp
import jax.experimental.pallas as pl
import jax.experimental.pallas.tpu as pltpu

S, D, F, H = 2048, 640, 1536, 32
DH = D // H
LANES = 128
BQ = 512
BK = 128
NQ = S // BQ
NG = D // LANES
NGS = 2 * NG - 1
MV = 24
BF = 512
UNROLL = 4
EPS = 1e-5
Q_SCALE = DH ** -0.5 * math.log2(math.e)

F32 = jnp.float32
BF16 = jnp.bfloat16
NT = (((1,), (1,)), ((), ()))


def _dot(a, b):
    return jax.lax.dot_general(a, b, (((1,), (0,)), ((), ())), preferred_element_type=F32)


def _kernel(x_hbm, wqkv_hbm, wo_hbm, wg_hbm, wu_hbm, wd_hbm, out_hbm,
            x_v, wqkv_v, wo_v, wg_v, wu_v, wd_v, xn_v, wt_v, kg_v, qt_v, vt_v,
            s_v, m_v, ot_v, out_v, x_sem, w_sem, o_sem):

    def x_copy(r):
        rows = pl.ds(r * BQ, BQ)
        return pltpu.make_async_copy(x_hbm.at[rows], x_v.at[rows], x_sem.at[r])

    def qkv_copy(i):
        cols = pl.ds(i * D, D)
        return pltpu.make_async_copy(wqkv_hbm.at[:, cols], wqkv_v.at[:, cols], w_sem.at[i])

    late_copies = [
        pltpu.make_async_copy(src, dst, w_sem.at[3 + i])
        for i, (src, dst) in enumerate(
            [(wg_hbm, wg_v), (wu_hbm, wu_v), (wd_hbm, wd_v), (wo_hbm, wo_v)])
    ]

    def out_copy(r):
        rows = pl.ds(pl.multiple_of(r * BF, BF), BF)
        return pltpu.make_async_copy(out_v.at[rows], out_hbm.at[rows], o_sem.at[r])

    def layer_norm(r):
        rows = pl.ds(pl.multiple_of(r * BQ, BQ), BQ)
        x = x_v[rows, :].astype(F32)
        mean = jnp.sum(x, axis=1, keepdims=True) * (1.0 / D)
        xc = x - mean
        var = jnp.sum(xc * xc, axis=1, keepdims=True) * (1.0 / D)
        xn_v[rows, :] = (xc * jax.lax.rsqrt(var + EPS)).astype(BF16)

    def k_proj(r):
        rows = pl.ds(pl.multiple_of(r * BQ, BQ), BQ)
        k = _dot(xn_v[rows, :], wqkv_v[:, D:2 * D])
        upper = jax.lax.broadcasted_iota(jnp.int32, (BQ, LANES), 1) >= LANES // 2
        for g in range(NG):
            kg = k[:, g * LANES:(g + 1) * LANES]
            kg_v[2 * g, rows, :] = kg.astype(BF16)
            if g + 1 < NG:
                nxt = k[:, (g + 1) * LANES:(g + 2) * LANES]
                kg_v[2 * g + 1, rows, :] = jnp.where(upper, kg, nxt).astype(BF16)

    x_copy(0).start()
    qkv_copy(1).start()
    x_copy(0).wait()
    for r in range(1, NQ):
        x_copy(r).start()
    qkv_copy(0).start()
    qkv_copy(2).start()
    layer_norm(0)
    qkv_copy(1).wait()

    def ln_k(r, carry):
        x_copy(r + 1).wait()
        k_proj(r)
        layer_norm(r + 1)
        return carry

    jax.lax.fori_loop(0, NQ - 1, ln_k, 0)

    qkv_copy(0).wait()
    qkv_copy(2).wait()
    for c in late_copies:
        c.start()
    k_proj(NQ - 1)
    for i in range(NG):
        wt_v[i * LANES:(i + 1) * LANES, :] = wqkv_v[:, i * LANES:(i + 1) * LANES].T
        wt_v[D + i * LANES:D + (i + 1) * LANES, :] = (
            wqkv_v[:, 2 * D + i * LANES:2 * D + (i + 1) * LANES].T)

    def q_v(r, carry):
        rows = pl.ds(pl.multiple_of(r * BQ, BQ), BQ)
        xn = xn_v[rows, :]
        qt = jax.lax.dot_general(wt_v[0:D, :], xn, NT, preferred_element_type=F32) * Q_SCALE
        upper = jax.lax.broadcasted_iota(jnp.int32, (LANES, BQ), 0) >= LANES // 2
        for g in range(NG):
            qg = qt[g * LANES:(g + 1) * LANES, :]
            qt_v[r, 2 * g] = qg.astype(BF16)
            if g + 1 < NG:
                nxt = qt[(g + 1) * LANES:(g + 2) * LANES, :]
                qt_v[r, 2 * g + 1] = jnp.where(upper, qg, nxt).astype(BF16)
        vt = jax.lax.dot_general(wt_v[D:2 * D, :], xn, NT, preferred_element_type=F32)
        vt = vt.astype(BF16).astype(F32)
        low = jax.lax.broadcasted_iota(jnp.int32, (8, BQ), 0) < 4
        for p in range(H // 2):
            b = 2 * DH * p
            mid = vt[b + 16:b + 24, :]
            vt_v[r, 2 * p, 0:16, :] = vt[b:b + 16, :]
            vt_v[r, 2 * p, 16:24, :] = jnp.where(low, mid, 1.0)
            vt_v[r, 2 * p + 1, 0:8, :] = jnp.where(low, 1.0, mid)
            vt_v[r, 2 * p + 1, 8:24, :] = vt[b + 24:b + 40, :]
        return carry

    jax.lax.fori_loop(0, NQ, q_v, 0)

    def head_operands(qb, h):
        lo = h * DH
        start = lo & (LANES - 1)
        gid = 2 * (lo >> 7) + (start > LANES - DH).astype(jnp.int32)
        row = jax.lax.broadcasted_iota(jnp.int32, (LANES, BQ), 0)
        mine = ((row - start) & (LANES - 1)) < DH
        qm = jnp.where(mine, qt_v[qb, gid].astype(F32), 0.0).astype(BF16)
        return gid, qm

    def scores_chunk(c, gid, qm):
        keys = pl.ds(c * BK, BK)
        st = _dot(kg_v[gid, keys, :], qm)
        s_v[keys, :] = st
        return jnp.max(st.reshape(BK // 8, 8, BQ), axis=0)

    def stage(h, nxt):
        m = jnp.max(m_v[...], axis=0, keepdims=True)
        gid, qm = head_operands(*nxt)
        mx = acc = None
        for c in range(S // BK):
            s = s_v[pl.ds(c * BK, BK), :]
            t = scores_chunk(c, gid, qm)
            mx = t if mx is None else jnp.maximum(mx, t)
            p = jnp.exp2(s - m).astype(BF16)
            r, off = divmod(c * BK, BQ)
            d = _dot(vt_v[r, h, :, off:off + BK], p)
            acc = d if acc is None else acc + d
        m_v[...] = mx
        return acc

    gid0, qm0 = head_operands(0, jnp.int32(0))
    mx0 = None
    for c in range(S // BK):
        t0 = scores_chunk(c, gid0, qm0)
        mx0 = t0 if mx0 is None else jnp.maximum(mx0, t0)
    m_v[...] = mx0

    n_pairs = NQ * H // 2

    def pair(t):
        qb, p = t >> 4, t & (H // 2 - 1)
        t1 = jnp.minimum(t + 1, n_pairs - 1)
        oa = stage(2 * p, (qb, 2 * p + 1))
        ob = stage(2 * p + 1, (t1 >> 4, 2 * (t1 & (H // 2 - 1))))
        oa = oa * (1.0 / oa[20:21, :])
        ob = ob * (1.0 / ob[0:1, :])
        low = jax.lax.broadcasted_iota(jnp.int32, (8, BQ), 0) < 4
        base = pl.multiple_of(p * 2 * DH, 8)
        ot_v[qb, pl.ds(base, 16), :] = oa[0:16]
        ot_v[qb, pl.ds(base + 16, 8), :] = jnp.where(low, oa[16:24], ob[0:8])
        ot_v[qb, pl.ds(base + 24, 16), :] = ob[8:24]

    def pairs(i, carry):
        for u in range(UNROLL):
            pair(i * UNROLL + u)
        return carry

    jax.lax.fori_loop(0, n_pairs // UNROLL, pairs, 0)

    for c in late_copies:
        c.wait()

    def finish(r, carry):
        rows = pl.ds(pl.multiple_of(r * BF, BF), BF)
        xn = xn_v[rows, :]
        g = _dot(xn, wg_v[...])
        u = _dot(xn, wu_v[...])
        hid = (g * jax.nn.sigmoid(g) * u).astype(BF16)
        o = ot_v[r].T.astype(BF16)
        y = x_v[rows, :].astype(F32) + _dot(o, wo_v[...]) + _dot(hid, wd_v[...])
        out_v[rows, :] = y.astype(BF16)
        out_copy(r).start()
        return carry

    jax.lax.fori_loop(0, S // BF, finish, 0)
    for r in range(S // BF):
        out_copy(r).wait()


@jax.jit
def pallas_parallel_sum__softmax_full_mha__swiglu_ffn__prompt_kernel(
    A_x: jax.Array,
    A_wqkv: jax.Array,
    A_wo: jax.Array,
    B_x: jax.Array,
    B_w_gate: jax.Array,
    B_w_up: jax.Array,
    B_w_down: jax.Array,
):
    del B_x
    hbm = pl.BlockSpec(memory_space=pl.ANY)
    out = pl.pallas_call(
        _kernel,
        out_shape=jax.ShapeDtypeStruct((S, D), BF16),
        in_specs=[hbm] * 6,
        out_specs=hbm,
        scratch_shapes=[
            pltpu.VMEM((S, D), BF16),
            pltpu.VMEM((D, 3 * D), BF16),
            pltpu.VMEM((D, D), BF16),
            pltpu.VMEM((D, F), BF16),
            pltpu.VMEM((D, F), BF16),
            pltpu.VMEM((F, D), BF16),
            pltpu.VMEM((S, D), BF16),
            pltpu.VMEM((2 * D, D), BF16),
            pltpu.VMEM((NGS, S, LANES), BF16),
            pltpu.VMEM((NQ, NGS, LANES, BQ), BF16),
            pltpu.VMEM((NQ, H, MV, BQ), F32),
            pltpu.VMEM((S, BQ), F32),
            pltpu.VMEM((8, BQ), F32),
            pltpu.VMEM((NQ, D, BQ), F32),
            pltpu.VMEM((S, D), BF16),
            pltpu.SemaphoreType.DMA((NQ,)),
            pltpu.SemaphoreType.DMA((7,)),
            pltpu.SemaphoreType.DMA((S // BF,)),
        ],
        compiler_params=pltpu.CompilerParams(
            vmem_limit_bytes=100 * 2**20,
            flags={"XLA_TPU_EVENLY_DISTRIBUTE_CRITICAL_NODES": True},
        ),
    )(A_x.reshape(S, D), A_wqkv, A_wo, B_w_gate, B_w_up, B_w_down)
    return out.reshape(1, S, D)
```
